```python
import os as _os
_os.environ.setdefault("JAX_PLATFORMS", "cpu")
import jax
import jax.numpy as jnp

def _softmax(x, axis=-1):
    return jax.nn.softmax(x, axis=axis)
def _gelu(x):
    return jax.nn.gelu(x, approximate=True)
def _silu(x):
    return jax.nn.silu(x)
def _sigmoid(x):
    return jax.nn.sigmoid(x)
def _layernorm(x, axis=-1, eps=1e-5):
    m = jnp.mean(x, axis=axis, keepdims=True)
    v = jnp.var(x, axis=axis, keepdims=True)
    return (x - m) / jnp.sqrt(v + eps)
def _scatter_add(tgt, idx, src, axis=0):
    return tgt.at[idx].add(src)
def _segment_sum(src, seg, n):
    return jax.ops.segment_sum(src, seg, n)
class _Rng:
    def __init__(self, key):
        self._k = key
    def _next(self):
        self._k, sub = jax.random.split(self._k)
        return sub
    def normal(self, shape):
        return jax.random.normal(self._next(), shape, dtype=jnp.bfloat16)
    def randint(self, lo, hi, shape):
        return jax.random.randint(self._next(), shape, lo, hi, dtype=jnp.int32)
    def uniform(self, shape, lo=0.0, hi=1.0):
        return jax.random.uniform(self._next(), shape, jnp.bfloat16, lo, hi)
    def permutation(self, n):
        return jax.random.permutation(self._next(), n)


kernel_name = 'concat_heads__ssm_conv_h3__sliding_block__prompt'

def setup_inputs():
    _rng = _Rng(jax.random.key(int.from_bytes(__import__("os").urandom(4), "little")))
    _w = (lambda a: (lambda t: t.astype(jnp.bfloat16) if jnp.issubdtype(t.dtype, jnp.floating) else t)(jnp.asarray(a)))
    def _A_setup():
        B, S, D = 1, 2048, 512
        ks = 4
        return {
            "q": _w((lambda *s: _rng.normal(s) * 0.05)(B, S, D)),
            "k": _w((lambda *s: _rng.normal(s) * 0.2)(B, S, D)),
            "v": _w((lambda *s: _rng.normal(s) * 0.2)(B, S, D)),
            "shift_k": _w((lambda *s: _rng.normal(s) * 0.2)(D, ks) * 0.5),
            "ssm_k": _w((lambda *s: _rng.normal(s) * 0.2)(D, S) * (1.0 / S ** 0.5)),
            "ssm_D": _w((lambda *s: _rng.normal(s) * 0.2)(D)),
        }
    _A_in = _A_setup()

    def _B_setup():
        B, S, D = 1, 2048, 512
        return {
            "x": _w((lambda *s: _rng.normal(s) * 0.2)(B, S, D)),
            "wqkv": _w((lambda *s: _rng.normal(s) * 0.2)(D, 3 * D)),
            "wo": _w((lambda *s: _rng.normal(s) * 0.05)(D, D)),
        }
    _B_in = _B_setup()

    return {
        "A_q": _A_in["q"],
        "A_k": _A_in["k"],
        "A_v": _A_in["v"],
        "A_shift_k": _A_in["shift_k"],
        "A_ssm_k": _A_in["ssm_k"],
        "A_ssm_D": _A_in["ssm_D"],
        "B_x": _B_in["x"],
        "B_wqkv": _B_in["wqkv"],
        "B_wo": _B_in["wo"],
    }

def reference(A_q, A_k, A_v, A_shift_k, A_ssm_k, A_ssm_D, B_x, B_wqkv, B_wo):
    def _A_ref(q, k, v, shift_k, ssm_k, ssm_D):
        B, S, D = q.shape
        ks = shift_k.shape[-1]
        k_pad = jnp.pad(k, ((0, 0), (ks - 1, 0), (0, 0)))
        k_shift = jnp.zeros_like(k)
        for t in range(ks):
            k_shift = k_shift + k_pad[:, t:t + S, :] * shift_k[:, ks - 1 - t][None, None, :]
        kv = k_shift * v
        L = 2 * S
        kv_pad = jnp.pad(kv, ((0, 0), (0, S), (0, 0)))
        kf_pad = jnp.pad(ssm_k, ((0, 0), (0, S)))
        kv_f = (lambda x, axes=(-2,-1): jnp.fft.rfft2(x.astype(jnp.float32), axes=axes))(kv_pad[:, None, :, :], axes=(1, 2))
        kf_f = (lambda x, axes=(-2,-1): jnp.fft.rfft2(x.astype(jnp.float32), axes=axes))(kf_pad[:, None, :], axes=(1, 2))
        kf_f = (lambda x, *d: x.transpose(*d))(kf_f, 1, 2, 0)
        y_f = kv_f * kf_f[None, :, :, :]
        y = (lambda x, s, axes=(-2,-1): jnp.fft.irfft2(x, s=s, axes=axes).astype(jnp.bfloat16))(y_f, (1, L), axes=(1, 2))[:, 0, :S, :]
        y = y + kv * ssm_D[None, None, :]
        return q * y

    def _B_ref(x, wqkv, wo):
        B, S, D = x.shape
        H = 32; Dh = D // H; W = 256
        qkv = (lambda x, *d: x.transpose(*d))((x @ wqkv).reshape(B, S, 3, H, Dh), 2, 0, 3, 1, 4)
        q, k, v = qkv[0], qkv[1], qkv[2]
        scores = jnp.einsum("bhqd,bhkd->bhqk", q, k) * (Dh ** -0.5)
        idx = jnp.arange(S)
        mask = (idx[:, None] - idx[None, :] >= 0) & (idx[:, None] - idx[None, :] < W)
        scores = jnp.where(mask[None, None], scores, -1e9)
        p = _softmax(scores, axis=-1)
        o = jnp.einsum("bhqk,bhkd->bhqd", p, v)
        return (lambda x, *d: x.transpose(*d))(o, 0, 2, 1, 3).reshape(B, S, D) @ wo

    a = _A_ref(A_q, A_k, A_v, A_shift_k, A_ssm_k, A_ssm_D)
    b = _B_ref(B_x, B_wqkv, B_wo)
    return jnp.concatenate([a, b], axis=-1)
```

```python
import numpy as np
import jax
import jax.numpy as jnp
import jax.experimental.pallas as pl
import jax.experimental.pallas.tpu as pltpu

S, D, H, DH = 2048, 512, 32, 16
N1, N2 = 32, 64
P = 72
BF = jnp.bfloat16
F32 = jnp.float32


def _consts():
    f1 = np.arange(N1)[:, None] + 0.25
    a = np.exp(-2j * np.pi * f1 * np.arange(N1)[None, :] / N1)
    w1 = np.stack([a.real, a.imag], 1).reshape(2 * N1, N1)
    ai = np.conj(a).T / S
    w1i = np.stack([ai.real, -ai.imag], 2).reshape(N1, 2 * N1)
    t2 = np.arange(N2)
    m = np.exp(-2j * np.pi * (f1[:, :, None] * t2[None, None, :] / S
                              + t2[:, None][None] * t2[None, None, :] / N2))
    def blk(c):
        return np.concatenate([np.concatenate([c.real, -c.imag], 2),
                               np.concatenate([c.imag, c.real], 2)], 1)
    return w1, w1i, blk(m), blk(np.conj(m).transpose(0, 2, 1))


def _dot(a, b):
    return jnp.dot(a, b, preferred_element_type=F32)


def _kernel(q_h, k_h, v_h, sh_r, sk_h, sd_r, x_h, wqkv_h, wo_h, w1_r, w1i_r, m_h, g_h,
            o_h, kk, qt, vt, ot, kv, kf, za, zb,
            x_r, wqkv_r, wo_r, k_r, v_r, sk_r, m_r, g_r, q_r, o_r, sems):
    cps = [pltpu.make_async_copy(a, b, sems.at[i]) for i, (a, b) in enumerate(
        [(x_h, x_r), (wqkv_h, wqkv_r), (wo_h, wo_r), (k_h, k_r), (v_h, v_r),
         (sk_h, sk_r), (m_h, m_r), (g_h, g_r), (q_h, q_r)])]
    cps[0].start()
    cps[1].start()
    cps[0].wait()
    cps[1].wait()
    for c in cps[2:]:
        c.start()
    ob = pltpu.make_async_copy(o_r.at[:, pl.ds(D, D)], o_h.at[:, pl.ds(D, D)], sems.at[9])
    oa = pltpu.make_async_copy(o_r.at[:, pl.ds(0, D)], o_h.at[:, pl.ds(0, D)], sems.at[10])
    xb = x_r[...]
    nt = (((1,), (1,)), ((), ()))
    kk[...] = _dot(xb, wqkv_r[:, D:2 * D]).astype(BF)
    wq = wqkv_r[:, 0:D].T
    qt[...] = (jax.lax.dot_general(wq, xb, nt, preferred_element_type=F32)
               * (0.25 * 1.4426950408889634)).astype(BF)
    wv = wqkv_r[:, 2 * D:].T
    vt[...] = jax.lax.dot_general(wv, xb, nt, preferred_element_type=F32).astype(BF)

    row = jax.lax.broadcasted_iota(jnp.int32, (128, 128), 0)
    col = jax.lax.broadcasted_iota(jnp.int32, (128, 128), 1)
    low = row > col

    def attn(i, g, case):
        q0 = pl.multiple_of(i * 128, 128)
        g0 = pl.multiple_of(g * 128, 128)
        qg = qt[pl.ds(g0, 128), pl.ds(q0, 128)]
        nk = (128, 256, 384)[case]
        k0 = pl.multiple_of(q0 - (nk - 128), 128)
        kb = kk[pl.ds(k0, nk), pl.ds(g0, 128)]
        outs = []
        qa = jnp.concatenate([jnp.where(row // DH == h, qg, jnp.zeros_like(qg))
                              for h in range(8)], 1)
        sa = _dot(kb, qa)
        for h in range(8):
            s = sa[:, h * 128:(h + 1) * 128]
            hi = s[nk - 128:]
            if case == 2:
                t = jnp.where(low, s[:128], hi)
            else:
                t = jnp.where(low, -1e30, hi)
            mx = jnp.max(t, axis=0, keepdims=True)
            if case >= 1:
                mid = s[nk - 256:nk - 128]
                mx = jnp.maximum(mx, jnp.max(mid, axis=0, keepdims=True))
            t = jnp.exp2(t - mx)
            l = jnp.sum(t, axis=0, keepdims=True)
            tb = t.astype(BF)
            if case == 0:
                p = tb
            else:
                mid = jnp.exp2(mid - mx)
                l = l + jnp.sum(mid, axis=0, keepdims=True)
                if case == 1:
                    p = jnp.concatenate([mid.astype(BF), tb], 0)
                else:
                    z = jnp.zeros_like(tb)
                    p = jnp.concatenate([jnp.where(low, tb, z), mid.astype(BF),
                                         jnp.where(low, z, tb)], 0)
            vh = vt[pl.ds(g0 + h * DH, DH), pl.ds(k0, nk)]
            outs.append(_dot(vh, p) * (1.0 / l))
        ot[pl.ds(g0, 128), pl.ds(q0, 128)] = jnp.concatenate(outs, 0).astype(BF)

    def b01(g, c):
        attn(0, g, 0)
        attn(1, g, 1)
        return c
    jax.lax.fori_loop(0, 4, b01, 0)

    def b2(n, c):
        attn(2 + n // 4, n % 4, 2)
        return c
    jax.lax.fori_loop(0, 14 * 4, b2, 0, unroll=4)
    for c in cps[2:]:
        c.wait()
    o_r[:, D:] = jax.lax.dot_general(ot[...], wo_r[...], (((0,), (0,)), ((), ())),
                                     preferred_element_type=F32).astype(BF)

    ob.start()
    kx = k_r[...].astype(F32)
    rows = jax.lax.broadcasted_iota(jnp.int32, (S, D), 0)
    sh = sh_r[...].astype(F32)
    acc = kx * sh[0:1]
    for j in range(1, 4):
        acc = acc + jnp.where(rows >= j, pltpu.roll(kx, j, 0), 0.0) * sh[j:j + 1]
    def ld(ref, rs):
        return jnp.concatenate([ref[c, rs, :] for c in range(4)], 1)

    def st(ref, rs, val):
        for c in range(4):
            ref[c, rs, :] = val[:, c * 128:(c + 1) * 128]

    kvb = acc.astype(BF) * v_r[...]
    kvf = kvb.astype(F32)
    skt = sk_r[...].astype(F32).T
    for i in range(N1):
        st(kv, pl.ds(i * P, N2), kvf[i * N2:(i + 1) * N2])
        st(kf, pl.ds(i * P, N2), skt[i * N2:(i + 1) * N2])

    def ld2(ref, f):
        return jnp.concatenate([ld(ref, pl.ds(pl.multiple_of((2 * f + j) * P, 8), N2))
                                for j in range(2)], 0)
    w1 = w1_r[...]
    w1i = w1i_r[...]

    def s1(t2, c):
        o, i = pl.ds(t2, 2 * N1, stride=P), pl.ds(t2, N1, stride=P)
        st(za, o, _dot(w1, ld(kv, i).astype(BF)))
        st(zb, o, _dot(w1, ld(kf, i).astype(BF)))
        return c
    jax.lax.fori_loop(0, N2, s1, 0, unroll=4)

    def s2(f, c):
        m = m_r[f]
        a = _dot(m, ld2(za, f).astype(BF))
        b = _dot(m, ld2(zb, f).astype(BF))
        ar, ai, br, bi = a[:64], a[64:], b[:64], b[64:]
        p = jnp.concatenate([ar * br - ai * bi, ar * bi + ai * br], 0)
        r = _dot(g_r[f], p.astype(BF))
        for j in range(2):
            st(za, pl.ds(pl.multiple_of((2 * f + j) * P, 8), N2), r[j * N2:(j + 1) * N2])
        return c
    jax.lax.fori_loop(0, N1, s2, 0, unroll=8)

    def s3(t2, c):
        st(kf, pl.ds(t2, N1, stride=P),
           _dot(w1i, ld(za, pl.ds(t2, 2 * N1, stride=P)).astype(BF)))
        return c
    jax.lax.fori_loop(0, N2, s3, 0, unroll=4)
    y = jnp.concatenate([ld(kf, pl.ds(i * P, N2)) for i in range(N1)], 0)
    y = y.astype(BF) + kvb * sd_r[...]
    o_r[:, :D] = q_r[...] * y
    oa.start()
    ob.wait()
    oa.wait()


@jax.jit
def pallas_concat_heads__ssm_conv_h3__sliding_block__prompt_kernel(
    A_q, A_k, A_v, A_shift_k, A_ssm_k, A_ssm_D, B_x, B_wqkv, B_wo):
    cs = [jnp.asarray(c.astype(np.float32)).astype(BF) for c in _consts()]
    out = pl.pallas_call(
        _kernel,
        out_shape=jax.ShapeDtypeStruct((S, 2 * D), BF),
        scratch_shapes=[pltpu.VMEM((S, D), BF), pltpu.VMEM((D, S), BF), pltpu.VMEM((D, S), BF),
                        pltpu.VMEM((D, S), BF), pltpu.VMEM((4, N1 * P, 128), F32), pltpu.VMEM((4, N1 * P, 128), F32),
                        pltpu.VMEM((4, 2 * N1 * P, 128), F32), pltpu.VMEM((4, 2 * N1 * P, 128), F32),
                        pltpu.VMEM((S, D), BF), pltpu.VMEM((D, 3 * D), BF), pltpu.VMEM((D, D), BF),
                        pltpu.VMEM((S, D), BF), pltpu.VMEM((S, D), BF), pltpu.VMEM((D, S), BF),
                        pltpu.VMEM((N1, 128, 128), BF), pltpu.VMEM((N1, 128, 128), BF),
                        pltpu.VMEM((S, D), BF), pltpu.VMEM((S, 2 * D), BF),
                        pltpu.SemaphoreType.DMA((11,))],
        in_specs=[pl.BlockSpec(memory_space=pltpu.VMEM if i in (3, 5, 9, 10) else pl.ANY)
                  for i in range(13)],
        out_specs=pl.BlockSpec(memory_space=pl.ANY),
        compiler_params=pltpu.CompilerParams(vmem_limit_bytes=110 * 1024 * 1024),
    )(A_q[0], A_k[0], A_v[0], A_shift_k.T, A_ssm_k, A_ssm_D[None], B_x[0], B_wqkv, B_wo, *cs)
    return out[None]
```
